```python
import jax
import jax.numpy as jnp

def _softmax(x, axis=-1):
    return jax.nn.softmax(x, axis=axis)
def _gelu(x):
    return jax.nn.gelu(x, approximate=True)
def _silu(x):
    return jax.nn.silu(x)
def _sigmoid(x):
    return jax.nn.sigmoid(x)
def _layernorm(x, axis=-1, eps=1e-5):
    m = jnp.mean(x, axis=axis, keepdims=True)
    v = jnp.var(x, axis=axis, keepdims=True)
    return (x - m) / jnp.sqrt(v + eps)
def _scatter_add(tgt, idx, src, axis=0):
    return tgt.at[idx].add(src)
def _segment_sum(src, seg, n):
    return jax.ops.segment_sum(src, seg, n)
class _Rng:
    def __init__(self, key):
        self._k = key
    def _next(self):
        self._k, sub = jax.random.split(self._k)
        return sub
    def normal(self, shape):
        return jax.random.normal(self._next(), shape, dtype=jnp.bfloat16)
    def randint(self, lo, hi, shape):
        return jax.random.randint(self._next(), shape, lo, hi, dtype=jnp.int32)
    def uniform(self, shape, lo=0.0, hi=1.0):
        return jax.random.uniform(self._next(), shape, jnp.bfloat16, lo, hi)
    def permutation(self, n):
        return jax.random.permutation(self._next(), n)


kernel_name = 'standalone__detection_seg_fpn_lateral__vision'

def setup_inputs():
    _rng = _Rng(jax.random.key(int.from_bytes(__import__("os").urandom(4), "little")))
    _w = (lambda a: (lambda t: t.astype(jnp.bfloat16) if jnp.issubdtype(t.dtype, jnp.floating) else t)(jnp.asarray(a)))
    H = W = (384 // 2) * 2
    C = 384
    k = 1
    return {
        "c_fine": _w((lambda *s: _rng.normal(s) * 0.05)(1, H, W, C)),
        "p_coarse": _w((lambda *s: _rng.normal(s) * 0.05)(1, H // 2, W // 2, C)),
        "w_lat": _w((lambda *s: _rng.normal(s) * 0.05)(C, C)),
        "w_out": _w((lambda *s: _rng.normal(s) * 0.05)(k, k, C, C)),
    }

def reference(c_fine, p_coarse, w_lat, w_out):
    B, H, W, C = c_fine.shape
    k = 1
    lat = jnp.einsum("bhwc,cd->bhwd", c_fine, w_lat)
    up = jnp.repeat(jnp.repeat(p_coarse, 2, axis=1), 2, axis=2)
    m = lat + up
    pad = k // 2
    mp = jnp.pad(m, ((0, 0), (pad, pad), (pad, pad), (0, 0)))
    o = None
    for di in range(k):
        for dj in range(k):
            t = jnp.einsum("bhwc,cd->bhwd", mp[:, di:di + H, dj:dj + W, :], w_out[di, dj])
            o = t if o is None else o + t
    return o
```

```python
import jax
import jax.numpy as jnp
import jax.experimental.pallas as pl
import jax.experimental.pallas.tpu as pltpu

_SLAB = 1024
_CHUNK_H = 8
_P_SLOTS = 20
_LEAD = 3
_SWITCH = 28
_W_LEAD = 2
_PIECE = 16


@jax.jit
def pallas_standalone__detection_seg_fpn_lateral__vision_kernel(
    c_fine: jax.Array,
    p_coarse: jax.Array,
    w_lat: jax.Array,
    w_out: jax.Array,
):
    B, H, W, C = c_fine.shape
    assert B == 1 and w_out.shape == (1, 1, C, C)
    assert p_coarse.shape == (1, H // 2, W // 2, C)
    n_chunks = H // _CHUNK_H
    chunk_px = _CHUNK_H * W
    spc = chunk_px // _SLAB
    n_slabs = n_chunks * spc
    n_units = n_chunks // 2
    half_w = W // 2
    assert spc * _SLAB == chunk_px and n_units * 2 * _CHUNK_H == H and W % 128 == 0

    def kernel(c_hbm, p_hbm, wl_hbm, wo_hbm, o_hbm,
               buf, pbuf, wl_v, wo_v, wf_v, c_sem, p_sem, w_sem, o_sem):
        def c_read(i):
            rows = pl.ds(spc * i, spc)
            return pltpu.make_async_copy(c_hbm.at[rows], buf.at[rows], c_sem.at[i])

        def p_read(i):
            return pltpu.make_async_copy(p_hbm.at[i], pbuf.at[i % _P_SLOTS], p_sem.at[i])

        def write_unit(u):
            rows = pl.ds(2 * spc * u, 2 * spc)
            for j in range(_SLAB // _PIECE):
                px = pl.ds(j * _PIECE, _PIECE)
                pltpu.make_async_copy(buf.at[rows, px], o_hbm.at[rows, px], o_sem).start()

        def compute(i):
            slot = i % _P_SLOTS
            x = pltpu.bitcast(buf[pl.ds(spc * i, spc)].reshape(chunk_px, C), jnp.uint32)
            for a in range(_CHUNK_H // 2):
                q = jnp.dot(pbuf[slot, pl.ds(half_w * a, half_w)], wo_v[...],
                            preferred_element_type=jnp.float32)
                for h in (2 * a, 2 * a + 1):
                    xr = x[half_w * h:half_w * (h + 1)]
                    ys = []
                    for parity in range(2):
                        xs = pltpu.unpack_elementwise(
                            xr, index=parity, packed_dtype=jnp.bfloat16,
                            unpacked_dtype=jnp.float32).astype(jnp.bfloat16)
                        ys.append(jnp.dot(xs, wf_v[...],
                                          preferred_element_type=jnp.float32) + q)
                    o = pltpu.bitcast(
                        pltpu.pack_elementwise(ys, packed_dtype=jnp.bfloat16), jnp.bfloat16)
                    for g in range(W // 128):
                        px = W * h + 128 * g
                        buf[spc * i + px // _SLAB, pl.ds(px % _SLAB, 128)] = (
                            o[128 * g:128 * (g + 1)])

        wl_copy = pltpu.make_async_copy(wl_hbm, wl_v, w_sem.at[0])
        wo_copy = pltpu.make_async_copy(wo_hbm, wo_v, w_sem.at[1])
        wl_copy.start()
        wo_copy.start()
        for i in range(_LEAD):
            p_read(i).start()
            c_read(i).start()
        wl_copy.wait()
        wo_copy.wait()
        wf_v[...] = jnp.dot(wl_v[...], wo_v[...],
                            preferred_element_type=jnp.float32).astype(jnp.bfloat16)

        @pl.loop(0, _SWITCH)
        def _read_phase(i):
            c_read(i).wait()
            p_read(i).wait()
            for t in range(2):
                j = _LEAD + 2 * i + t
                pl.when(j < _P_SLOTS)(lambda: p_read(j).start())
                pl.when(j < n_chunks)(lambda: c_read(j).start())
            compute(i)
            pl.when(i + _P_SLOTS < n_chunks)(lambda: p_read(i + _P_SLOTS).start())

        @pl.loop(_SWITCH, n_chunks)
        def _drain_reads(i):
            c_read(i).wait()
            p_read(i).wait()

        pl.loop(0, _W_LEAD)(write_unit)

        @pl.loop(_SWITCH, n_chunks)
        def _write_phase(i):
            u = _W_LEAD + i - _SWITCH
            pl.when(u < n_units - 1)(lambda: write_unit(u))
            compute(i)

        pl.loop(min(_W_LEAD + n_chunks - _SWITCH, n_units - 1), n_units)(write_unit)
        pltpu.make_async_copy(buf, o_hbm, o_sem).wait()

    assert _SWITCH + _P_SLOTS >= n_chunks and _LEAD + 2 * _SWITCH >= n_chunks
    assert all(2 * (_W_LEAD + i - _SWITCH + 1) <= i for i in range(_SWITCH, n_chunks)
               if _W_LEAD + i - _SWITCH < n_units - 1)

    out = pl.pallas_call(
        kernel,
        in_specs=[pl.BlockSpec(memory_space=pl.ANY)] * 4,
        out_specs=pl.BlockSpec(memory_space=pl.ANY),
        out_shape=jax.ShapeDtypeStruct((n_slabs, _SLAB, C), c_fine.dtype),
        scratch_shapes=[
            pltpu.VMEM((n_slabs, _SLAB, C), jnp.bfloat16),
            pltpu.VMEM((_P_SLOTS, chunk_px // 4, C), jnp.bfloat16),
            pltpu.VMEM((C, C), jnp.bfloat16),
            pltpu.VMEM((C, C), jnp.bfloat16),
            pltpu.VMEM((C, C), jnp.bfloat16),
            pltpu.SemaphoreType.DMA((n_chunks,)),
            pltpu.SemaphoreType.DMA((n_chunks,)),
            pltpu.SemaphoreType.DMA((2,)),
            pltpu.SemaphoreType.DMA(()),
        ],
        compiler_params=pltpu.CompilerParams(vmem_limit_bytes=127 * 2**20),
    )(
        c_fine.reshape(n_slabs, _SLAB, C),
        p_coarse.reshape(n_chunks, chunk_px // 4, C),
        w_lat,
        w_out.reshape(C, C),
    )
    return out.reshape(B, H, W, C)
```

```python
import jax
import jax.numpy as jnp
import jax.experimental.pallas as pl
import jax.experimental.pallas.tpu as pltpu

_SLAB = 2048
_CHUNK_H = 16
_P_SLOTS = 12
_LEAD = 7
_RATE = 5
_READ_PX = (128, 128)
_PIECE = 16
_GROUPS = (0, 1, 2, 4, 7, 12, 16)


def _cuts(total):
    out, off = [], 0
    while off < total:
        n = min(_READ_PX[len(out) % len(_READ_PX)], total - off)
        out.append((off, n))
        off += n
    return out


def _spans(start, n, slab):
    out = []
    while n:
        k = min(n, slab - start % slab)
        out.append((start // slab, pl.ds(start % slab, k)))
        start += k
        n -= k
    return out


@jax.jit
def pallas_standalone__detection_seg_fpn_lateral__vision_kernel(
    c_fine: jax.Array,
    p_coarse: jax.Array,
    w_lat: jax.Array,
    w_out: jax.Array,
):
    B, H, W, C = c_fine.shape
    assert B == 1 and w_out.shape == (1, 1, C, C)
    assert p_coarse.shape == (1, H // 2, W // 2, C)
    half_w = W // 2
    n_chunks = H // _CHUNK_H
    spc = _CHUNK_H * W // _SLAB
    n_slabs = n_chunks * spc
    n_units = n_chunks // 2
    n_read = (n_slabs - _LEAD) // _RATE
    n_pieces = _SLAB // _PIECE
    p_ring = spc * _P_SLOTS
    bounds = _GROUPS + (n_chunks,)

    assert n_slabs * _SLAB == H * W and n_units * 2 == n_chunks
    assert _LEAD + _RATE * n_read == n_slabs
    assert all(s // spc - _P_SLOTS < (s - _LEAD) // _RATE for s in range(_LEAD, n_slabs))
    for lo, hi in zip(bounds, bounds[1:]):
        assert spc * hi <= _LEAD + _RATE * min(lo, n_read)
        assert lo % _P_SLOTS + hi - lo <= _P_SLOTS
    assert all(2 * (i - n_read) + 1 < i for i in range(n_read, n_chunks))

    def kernel(c_hbm, p_hbm, wl_hbm, wo_hbm, o_hbm,
               buf, pbuf, wl_v, wo_v, wf_v, c_sem, p_sem, w_sem, o_sem):
        def read_half_slab(s, half):
            group = sum((s >= spc * first).astype(jnp.int32) for first in _GROUPS[1:])
            copies = []
            for off, n in _cuts(_SLAB // 8):
                px = pl.ds(half * _SLAB // 8 + off, n)
                copies.append((p_hbm.at[s, px], pbuf.at[s % p_ring, px], p_sem.at[group]))
            for off, n in _cuts(_SLAB // 2):
                px = pl.ds(half * _SLAB // 2 + off, n)
                copies.append((c_hbm.at[s, px], buf.at[s, px], c_sem.at[group]))
            for k, refs in enumerate(copies):
                pltpu.make_async_copy(*refs).start(priority=k % 2)

        def wait_group(g):
            lo, n = spc * bounds[g], spc * (bounds[g + 1] - bounds[g])
            pltpu.make_async_copy(
                c_hbm.at[pl.ds(lo, n)], buf.at[pl.ds(lo, n)], c_sem.at[g]).wait()
            pltpu.make_async_copy(
                p_hbm.at[pl.ds(lo, n)], pbuf.at[pl.ds(lo % p_ring, n)], p_sem.at[g]).wait()

        def write_half_unit(u, half):
            rows = pl.ds(2 * spc * u, 2 * spc)
            for j in range(half * n_pieces // 2, (half + 1) * n_pieces // 2):
                px = pl.ds(j * _PIECE, _PIECE)
                pltpu.make_async_copy(
                    buf.at[rows, px], o_hbm.at[rows, px], o_sem).start(priority=1)

        def compute_half_chunk(i, half):
            cv = buf.at[pl.ds(spc * i, spc)]
            pv = pbuf.at[pl.ds(spc * (i % _P_SLOTS), spc)]
            for a in range(half * _CHUNK_H // 4, (half + 1) * _CHUNK_H // 4):
                p = jnp.concatenate(
                    [pv[s, px] for s, px in _spans(half_w * a, half_w, _SLAB // 4)])
                q = jnp.dot(p, wo_v[...], preferred_element_type=jnp.float32)
                for h in (2 * a, 2 * a + 1):
                    where = _spans(W * h, W, _SLAB)
                    x = pltpu.bitcast(
                        jnp.concatenate([cv[s, px] for s, px in where]), jnp.uint32)
                    ys = []
                    for parity in range(2):
                        xs = pltpu.unpack_elementwise(
                            x, index=parity, packed_dtype=jnp.bfloat16,
                            unpacked_dtype=jnp.float32).astype(jnp.bfloat16)
                        ys.append(jnp.dot(xs, wf_v[...],
                                          preferred_element_type=jnp.float32) + q)
                    o = pltpu.bitcast(
                        pltpu.pack_elementwise(ys, packed_dtype=jnp.bfloat16), jnp.bfloat16)
                    off = 0
                    for s, px in where:
                        cv[s, px] = o[off:off + px.size]
                        off += px.size

        wl_copy = pltpu.make_async_copy(wl_hbm, wl_v, w_sem)
        wo_copy = pltpu.make_async_copy(wo_hbm, wo_v, w_sem)
        wl_copy.start()
        wo_copy.start()

        @pl.loop(0, _LEAD)
        def _prime(s):
            read_half_slab(s, 0)
            read_half_slab(s, 1)

        wl_copy.wait()
        wo_copy.wait()
        wf_v[...] = jnp.dot(wl_v[...], wo_v[...],
                            preferred_element_type=jnp.float32).astype(jnp.bfloat16)

        @pl.loop(0, n_chunks)
        def _step(i):
            for half in range(2):
                @pl.when(i < n_read)
                def _reads(half=half):
                    for t in range(half * _RATE, (half + 1) * _RATE):
                        read_half_slab(_LEAD + _RATE * i + t // 2, t % 2)

                @pl.when(i >= n_read)
                def _writes(half=half):
                    write_half_unit(i - n_read, half)

                if half == 0:
                    for g, first in enumerate(_GROUPS):
                        pl.when(i == first)(lambda g=g: wait_group(g))
                compute_half_chunk(i, half)

        @pl.loop(n_chunks - n_read, n_units)
        def _tail(u):
            write_half_unit(u, 0)
            write_half_unit(u, 1)

        pltpu.make_async_copy(buf, o_hbm, o_sem).wait()

    out = pl.pallas_call(
        kernel,
        in_specs=[pl.BlockSpec(memory_space=pl.ANY)] * 4,
        out_specs=pl.BlockSpec(memory_space=pl.ANY),
        out_shape=jax.ShapeDtypeStruct((n_slabs, _SLAB, C), c_fine.dtype),
        scratch_shapes=[
            pltpu.VMEM((n_slabs, _SLAB, C), jnp.bfloat16),
            pltpu.VMEM((p_ring, _SLAB // 4, C), jnp.bfloat16),
            pltpu.VMEM((C, C), jnp.bfloat16),
            pltpu.VMEM((C, C), jnp.bfloat16),
            pltpu.VMEM((C, C), jnp.bfloat16),
            pltpu.SemaphoreType.DMA((len(_GROUPS),)),
            pltpu.SemaphoreType.DMA((len(_GROUPS),)),
            pltpu.SemaphoreType.DMA(()),
            pltpu.SemaphoreType.DMA(()),
        ],
        compiler_params=pltpu.CompilerParams(
            vmem_limit_bytes=124 * 2**20, disable_bounds_checks=True),
    )(
        c_fine.reshape(n_slabs, _SLAB, C),
        p_coarse.reshape(n_slabs, _SLAB // 4, C),
        w_lat,
        w_out.reshape(C, C),
    )
    return out.reshape(B, H, W, C)
```

```python
import jax
import jax.numpy as jnp
import jax.experimental.pallas as pl
import jax.experimental.pallas.tpu as pltpu

_SLAB = 2048
_CHUNK_H = 16
_P_SLOTS = 12
_CELLS = 8
_LEAD = 23
_RATE = 13
_READ_PX = 32
_WRITE_PX = 16
_GROUPS = (0, 1, 2, 4, 7, 12, 16)


def _spans(start, n, slab):
    out = []
    while n:
        k = min(n, slab - start % slab)
        out.append((start // slab, pl.ds(start % slab, k)))
        start += k
        n -= k
    return out


@jax.jit
def pallas_standalone__detection_seg_fpn_lateral__vision_kernel(
    c_fine: jax.Array,
    p_coarse: jax.Array,
    w_lat: jax.Array,
    w_out: jax.Array,
):
    B, H, W, C = c_fine.shape
    assert B == 1 and w_out.shape == (1, 1, C, C)
    assert p_coarse.shape == (1, H // 2, W // 2, C)
    half_w = W // 2
    n_chunks = H // _CHUNK_H
    spc = _CHUNK_H * W // _SLAB
    n_slabs = n_chunks * spc
    n_units = n_chunks // 2
    n_cells = n_chunks * _CELLS
    n_read = (n_cells - _LEAD) // _RATE
    n_pieces = _SLAB // _WRITE_PX
    bounds = _GROUPS + (n_chunks,)

    assert n_slabs * _SLAB == H * W and n_units * 2 == n_chunks
    assert _LEAD + _RATE * n_read == n_cells
    assert all(d // _CELLS - _P_SLOTS < (d - _LEAD) // _RATE for d in range(_LEAD, n_cells))
    for lo, hi in zip(bounds, bounds[1:]):
        assert _CELLS * hi <= _LEAD + _RATE * min(lo, n_read)
        assert lo % _P_SLOTS + hi - lo <= _P_SLOTS
    assert all(2 * (i - n_read) + 1 < i for i in range(n_read, n_chunks))

    def kernel(c_hbm, p_hbm, wl_hbm, wo_hbm, o_hbm,
               buf, pbuf, wl_v, wo_v, wf_v, c_sem, p_sem, w_sem, o_sem):
        def read_cell(d):
            j, k = d // _CELLS, d % _CELLS
            group = sum((j >= first).astype(jnp.int32) for first in _GROUPS[1:])
            rows = pl.ds(spc * j, spc)
            for src, dst, dst_rows, sem, slab in (
                    (p_hbm, pbuf, pl.ds(spc * (j % _P_SLOTS), spc), p_sem, _SLAB // 4),
                    (c_hbm, buf, rows, c_sem, _SLAB)):
                width = slab // 2 // _CELLS
                for t in range(width // _READ_PX):
                    for queue in range(2):
                        start = queue * slab // 2 + k * width + t * _READ_PX
                        px = pl.ds(pl.multiple_of(start, _READ_PX), _READ_PX)
                        pltpu.make_async_copy(
                            src.at[rows, px], dst.at[dst_rows, px], sem.at[group]
                        ).start(priority=queue)

        def wait_group(g):
            rows = pl.ds(spc * bounds[g], spc * (bounds[g + 1] - bounds[g]))
            ring = pl.ds(spc * (bounds[g] % _P_SLOTS), rows.size)
            pltpu.make_async_copy(c_hbm.at[rows], buf.at[rows], c_sem.at[g]).wait()
            pltpu.make_async_copy(p_hbm.at[rows], pbuf.at[ring], p_sem.at[g]).wait()

        def write_part(u, h):
            rows = pl.ds(2 * spc * u, 2 * spc)
            for t in range(h * n_pieces // _CHUNK_H, (h + 1) * n_pieces // _CHUNK_H):
                px = pl.ds(t * _WRITE_PX, _WRITE_PX)
                pltpu.make_async_copy(
                    buf.at[rows, px], o_hbm.at[rows, px], o_sem).start(priority=1)

        def step(i, steps, queue_dmas):
            for g, first in enumerate(_GROUPS):
                if first in steps:
                    pl.when(i == first)(lambda g=g: wait_group(g))
            cv = buf.at[pl.ds(spc * i, spc)]
            pv = pbuf.at[pl.ds(spc * (i % _P_SLOTS), spc)]
            for a in range(_CHUNK_H // 2):
                p = jnp.concatenate(
                    [pv[s, px] for s, px in _spans(half_w * a, half_w, _SLAB // 4)])
                q = jnp.dot(p, wo_v[...], preferred_element_type=jnp.float32)
                for h in (2 * a, 2 * a + 1):
                    where = _spans(W * h, W, _SLAB)
                    x = pltpu.bitcast(
                        jnp.concatenate([cv[s, px] for s, px in where]), jnp.uint32)
                    queue_dmas(h)
                    ys = []
                    for parity in range(2):
                        xs = pltpu.unpack_elementwise(
                            x, index=parity, packed_dtype=jnp.bfloat16,
                            unpacked_dtype=jnp.float32).astype(jnp.bfloat16)
                        ys.append(jnp.dot(xs, wf_v[...],
                                          preferred_element_type=jnp.float32) + q)
                    o = pltpu.bitcast(
                        pltpu.pack_elementwise(ys, packed_dtype=jnp.bfloat16), jnp.bfloat16)
                    off = 0
                    for s, px in where:
                        cv[s, px] = o[off:off + px.size]
                        off += px.size

        wl_copy = pltpu.make_async_copy(wl_hbm, wl_v, w_sem)
        wo_copy = pltpu.make_async_copy(wo_hbm, wo_v, w_sem)
        wl_copy.start()
        wo_copy.start()
        pl.loop(0, _LEAD)(read_cell)
        wl_copy.wait()
        wo_copy.wait()
        wf_v[...] = jnp.dot(wl_v[...], wo_v[...],
                            preferred_element_type=jnp.float32).astype(jnp.bfloat16)

        @pl.loop(0, n_read)
        def _read_phase(i):
            def queue_dmas(h):
                for t in range(h * _RATE // _CHUNK_H, (h + 1) * _RATE // _CHUNK_H):
                    read_cell(_LEAD + _RATE * i + t)
            step(i, range(n_read), queue_dmas)

        @pl.loop(n_read, n_chunks)
        def _write_phase(i):
            step(i, range(n_read, n_chunks), lambda h: write_part(i - n_read, h))

        @pl.loop(n_chunks - n_read, n_units)
        def _tail(u):
            for h in range(_CHUNK_H):
                write_part(u, h)

        pltpu.make_async_copy(buf, o_hbm, o_sem).wait()

    out = pl.pallas_call(
        kernel,
        in_specs=[pl.BlockSpec(memory_space=pl.ANY)] * 4,
        out_specs=pl.BlockSpec(memory_space=pl.ANY),
        out_shape=jax.ShapeDtypeStruct((n_slabs, _SLAB, C), c_fine.dtype),
        scratch_shapes=[
            pltpu.VMEM((n_slabs, _SLAB, C), jnp.bfloat16),
            pltpu.VMEM((spc * _P_SLOTS, _SLAB // 4, C), jnp.bfloat16),
            pltpu.VMEM((C, C), jnp.bfloat16),
            pltpu.VMEM((C, C), jnp.bfloat16),
            pltpu.VMEM((C, C), jnp.bfloat16),
            pltpu.SemaphoreType.DMA((len(_GROUPS),)),
            pltpu.SemaphoreType.DMA((len(_GROUPS),)),
            pltpu.SemaphoreType.DMA(()),
            pltpu.SemaphoreType.DMA(()),
        ],
        compiler_params=pltpu.CompilerParams(
            vmem_limit_bytes=126 * 2**20, disable_bounds_checks=True),
    )(
        c_fine.reshape(n_slabs, _SLAB, C),
        p_coarse.reshape(n_slabs, _SLAB // 4, C),
        w_lat,
        w_out.reshape(C, C),
    )
    return out.reshape(B, H, W, C)
```

```python
import jax
import jax.numpy as jnp
import numpy as np
import jax.experimental.pallas as pl
import jax.experimental.pallas.tpu as pltpu

_SLAB = 2048
_CHUNK_H = 16
_P_SLOTS = 12
_CELLS = 8
_LEAD = 23
_RATE = 13
_READ_PX = 16
_WRITE_PX = 16
_GROUPS = (0, 1, 2, 4, 7, 12, 16)


def _spans(start, n, slab):
    out = []
    while n:
        k = min(n, slab - start % slab)
        out.append((start // slab, pl.ds(start % slab, k)))
        start += k
        n -= k
    return out


@jax.jit
def pallas_standalone__detection_seg_fpn_lateral__vision_kernel(
    c_fine: jax.Array,
    p_coarse: jax.Array,
    w_lat: jax.Array,
    w_out: jax.Array,
):
    B, H, W, C = c_fine.shape
    assert B == 1 and w_out.shape == (1, 1, C, C)
    assert p_coarse.shape == (1, H // 2, W // 2, C)
    half_w = W // 2
    n_chunks = H // _CHUNK_H
    spc = _CHUNK_H * W // _SLAB
    n_slabs = n_chunks * spc
    n_units = n_chunks // 2
    n_cells = n_chunks * _CELLS
    n_read = (n_cells - _LEAD) // _RATE
    n_pieces = _SLAB // _WRITE_PX
    bounds = _GROUPS + (n_chunks,)

    assert n_slabs * _SLAB == H * W and n_units * 2 == n_chunks
    assert _LEAD + _RATE * n_read == n_cells
    assert all(d // _CELLS - _P_SLOTS < (d - _LEAD) // _RATE for d in range(_LEAD, n_cells))
    for lo, hi in zip(bounds, bounds[1:]):
        assert _CELLS * hi <= _LEAD + _RATE * min(lo, n_read)
        assert lo % _P_SLOTS + hi - lo <= _P_SLOTS
    assert all(2 * (i - n_read) + 1 < i for i in range(n_read, n_chunks))

    def kernel(c_hbm, p_hbm, wl_hbm, wo_hbm, o_hbm,
               buf, pbuf, wl_v, wo_v, wf_v, c_sem, p_sem, w_sem, o_sem):
        def read_cell(d):
            j, k = d // _CELLS, d % _CELLS
            group = sum((j >= first).astype(jnp.int32) for first in _GROUPS[1:])
            rows = pl.ds(spc * j, spc)
            for src, dst, dst_rows, sem, slab in (
                    (p_hbm, pbuf, pl.ds(spc * (j % _P_SLOTS), spc), p_sem, _SLAB // 4),
                    (c_hbm, buf, rows, c_sem, _SLAB)):
                width = slab // 2 // _CELLS
                for t in range(width // _READ_PX):
                    for queue in range(2):
                        start = queue * slab // 2 + k * width + t * _READ_PX
                        px = pl.ds(pl.multiple_of(start, _READ_PX), _READ_PX)
                        pltpu.make_async_copy(
                            src.at[rows, px], dst.at[dst_rows, px], sem.at[group]
                        ).start(priority=queue)

        def wait_group(g):
            rows = pl.ds(spc * bounds[g], spc * (bounds[g + 1] - bounds[g]))
            ring = pl.ds(spc * (bounds[g] % _P_SLOTS), rows.size)
            pltpu.make_async_copy(c_hbm.at[rows], buf.at[rows], c_sem.at[g]).wait()
            pltpu.make_async_copy(p_hbm.at[rows], pbuf.at[ring], p_sem.at[g]).wait()

        def write_part(u, h):
            rows = pl.ds(2 * spc * u, 2 * spc)
            for t in range(h * n_pieces // _CHUNK_H, (h + 1) * n_pieces // _CHUNK_H):
                px = pl.ds(t * _WRITE_PX, _WRITE_PX)
                pltpu.make_async_copy(buf.at[rows, px], o_hbm.at[rows, px], o_sem).start()

        def project(bits, q):
            xs = jax.lax.bitcast_convert_type(bits, jnp.float32).astype(jnp.bfloat16)
            y = jnp.dot(xs, wf_v[...], preferred_element_type=jnp.float32) + q
            return jax.lax.bitcast_convert_type(
                y.astype(jnp.bfloat16).astype(jnp.float32), jnp.uint32)

        def step(i, steps, queue_dmas):
            for g, first in enumerate(_GROUPS):
                if first in steps:
                    pl.when(i == first)(lambda g=g: wait_group(g))
            cv = buf.at[pl.ds(spc * i, spc)]
            pv = pbuf.at[pl.ds(spc * (i % _P_SLOTS), spc)]
            for a in range(_CHUNK_H // 2):
                p = jnp.concatenate(
                    [pv[s, px] for s, px in _spans(half_w * a, half_w, _SLAB // 4)])
                q = jnp.dot(p, wo_v[...], preferred_element_type=jnp.float32)
                for h in (2 * a, 2 * a + 1):
                    where = _spans(W * h, W, _SLAB)
                    x = pltpu.bitcast(
                        jnp.concatenate([cv[s, px] for s, px in where]), jnp.uint32)
                    queue_dmas(h)
                    even = project(x << 16, q)
                    odd = project(x & np.uint32(0xFFFF0000), q)
                    o = pltpu.bitcast((even >> 16) | odd, jnp.bfloat16)
                    off = 0
                    for s, px in where:
                        cv[s, px] = o[off:off + px.size]
                        off += px.size

        wl_copy = pltpu.make_async_copy(wl_hbm, wl_v, w_sem)
        wo_copy = pltpu.make_async_copy(wo_hbm, wo_v, w_sem)
        wl_copy.start()
        wo_copy.start()
        pl.loop(0, _LEAD)(read_cell)
        wl_copy.wait()
        wo_copy.wait()
        wf_v[...] = jnp.dot(wl_v[...], wo_v[...],
                            preferred_element_type=jnp.float32).astype(jnp.bfloat16)

        @pl.loop(0, n_read)
        def _read_phase(i):
            def queue_dmas(h):
                for t in range(h * _RATE // _CHUNK_H, (h + 1) * _RATE // _CHUNK_H):
                    read_cell(_LEAD + _RATE * i + t)
            step(i, range(n_read), queue_dmas)

        @pl.loop(n_read, n_chunks)
        def _write_phase(i):
            step(i, range(n_read, n_chunks), lambda h: write_part(i - n_read, h))

        @pl.loop(n_chunks - n_read, n_units)
        def _tail(u):
            for h in range(_CHUNK_H):
                write_part(u, h)

        pltpu.make_async_copy(buf, o_hbm, o_sem).wait()

    out = pl.pallas_call(
        kernel,
        in_specs=[pl.BlockSpec(memory_space=pl.ANY)] * 4,
        out_specs=pl.BlockSpec(memory_space=pl.ANY),
        out_shape=jax.ShapeDtypeStruct((n_slabs, _SLAB, C), c_fine.dtype),
        scratch_shapes=[
            pltpu.VMEM((n_slabs, _SLAB, C), jnp.bfloat16),
            pltpu.VMEM((spc * _P_SLOTS, _SLAB // 4, C), jnp.bfloat16),
            pltpu.VMEM((C, C), jnp.bfloat16),
            pltpu.VMEM((C, C), jnp.bfloat16),
            pltpu.VMEM((C, C), jnp.bfloat16),
            pltpu.SemaphoreType.DMA((len(_GROUPS),)),
            pltpu.SemaphoreType.DMA((len(_GROUPS),)),
            pltpu.SemaphoreType.DMA(()),
            pltpu.SemaphoreType.DMA(()),
        ],
        compiler_params=pltpu.CompilerParams(
            vmem_limit_bytes=126 * 2**20, disable_bounds_checks=True),
    )(
        c_fine.reshape(n_slabs, _SLAB, C),
        p_coarse.reshape(n_slabs, _SLAB // 4, C),
        w_lat,
        w_out.reshape(C, C),
    )
    return out.reshape(B, H, W, C)
```
